```python
import os as _os
_os.environ.setdefault("JAX_PLATFORMS", "cpu")
import jax
import jax.numpy as jnp

def _softmax(x, axis=-1):
    return jax.nn.softmax(x, axis=axis)
def _gelu(x):
    return jax.nn.gelu(x, approximate=True)
def _silu(x):
    return jax.nn.silu(x)
def _sigmoid(x):
    return jax.nn.sigmoid(x)
def _layernorm(x, axis=-1, eps=1e-5):
    m = jnp.mean(x, axis=axis, keepdims=True)
    v = jnp.var(x, axis=axis, keepdims=True)
    return (x - m) / jnp.sqrt(v + eps)
def _scatter_add(tgt, idx, src, axis=0):
    return tgt.at[idx].add(src)
def _segment_sum(src, seg, n):
    return jax.ops.segment_sum(src, seg, n)
class _Rng:
    def __init__(self, key):
        self._k = key
    def _next(self):
        self._k, sub = jax.random.split(self._k)
        return sub
    def normal(self, shape):
        return jax.random.normal(self._next(), shape, dtype=jnp.bfloat16)
    def randint(self, lo, hi, shape):
        return jax.random.randint(self._next(), shape, lo, hi, dtype=jnp.int32)
    def uniform(self, shape, lo=0.0, hi=1.0):
        return jax.random.uniform(self._next(), shape, jnp.bfloat16, lo, hi)
    def permutation(self, n):
        return jax.random.permutation(self._next(), n)


kernel_name = 'standalone__gqa_block_cached__near_ridge'

def setup_inputs():
    _rng = _Rng(jax.random.key(int.from_bytes(__import__("os").urandom(4), "little")))
    _w = (lambda a: (lambda t: t.astype(jnp.bfloat16) if jnp.issubdtype(t.dtype, jnp.floating) else t)(jnp.asarray(a)))
    B, Sq, D = 8, 64, 512
    Hq, Hkv, Sk, Dh = 32, 8, 64, 128
    assert Hq % Hkv == 0, (Hq, Hkv)
    return {
        "x": _w((lambda *s: _rng.normal(s) * 0.8)(B, Sq, D)),
        "k_cache": _w((lambda *s: _rng.normal(s) * 0.8)(B, Hkv, Sk, Dh)),
        "v_cache": _w((lambda *s: _rng.normal(s) * 0.05)(B, Hkv, Sk, Dh)),
        "wq": _w((lambda *s: _rng.normal(s) * 0.8)(D, Hq * Dh) * (D ** -0.5)),
        "wo": _w((lambda *s: _rng.normal(s) * 0.05)(Hq * Dh, D) * ((Hq * Dh) ** -0.5)),
    }

def reference(x, k_cache, v_cache, wq, wo):
    B, Sq, D = x.shape
    Hq, Dh = 32, 128
    Hkv = k_cache.shape[1]
    rep = Hq // Hkv
    q = (lambda x, *d: x.transpose(*d))((x @ wq).reshape(B, Sq, Hq, Dh), 0, 2, 1, 3)
    k = jnp.repeat(k_cache, rep, axis=1)
    v = jnp.repeat(v_cache, rep, axis=1)
    scores = jnp.einsum("bhqd,bhkd->bhqk", q, k) * (Dh ** -0.5)
    p = _softmax(scores, axis=-1)
    o = jnp.einsum("bhqk,bhkd->bhqd", p, v)
    return (lambda x, *d: x.transpose(*d))(o, 0, 2, 1, 3).reshape(B, Sq, Hq * Dh) @ wo
```

```python
import functools
import jax
import jax.numpy as jnp
from jax import lax
from jax.experimental import pallas as pl
from jax.experimental.pallas import tpu as pltpu

B, SQ, D = 8, 64, 512
HQ, HKV, SK, DH = 32, 8, 64, 128
REP = HQ // HKV
GW = REP * DH
M = B * SQ
NT = 4

DMA_L = 0.60
DMA_R = 0.66
ORDER = "c"
KHEAD = True
C_PP = 0.145
C_AP = 0.27
C_A = 0.37
C_NEXT_A2 = 0.15


def _recip(l):
    r = pl.reciprocal(l, approx=True)
    return r * (2.0 - l * r)


UNIT_MB = {"x": 0.5, "wqt": 0.125, "wq": 0.5, "wo": 0.5, "k": 0.125, "v": 0.125, "xk": 0.125, "wqk": 0.125}
CHUNK_US = {"Q": 512 / 1500.0, "O": 512 / 1500.0, "QK": 512 / 1500.0, "A1": 40 / 1500.0, "A2": 64 / 1500.0}
PROJ = ("Q", "O", "QK")


def needs(op):
    kind, g, j = op
    if kind == "QK":
        return [("xk", j), ("wqk", j)]
    if kind == "Q":
        if g == 0:
            return [("x",), ("wqt", 0, j)]
        return [("wq", g)]
    if kind == "O":
        return [("wo", g)]
    if kind == "A1":
        return [("k", g)]
    if kind == "A2":
        return [("v", g)]
    raise ValueError(op)


def stage(s):
    proj = []
    for j in range(NT):
        if s + 1 < HKV:
            proj.append(("Q", s + 1, j))
        if s >= 1:
            proj.append(("O", s - 1, j))
    if s == HKV:
        return proj
    seq = []
    take = lambda: seq.append(proj.pop(0)) if proj else None
    a1 = [("A1", s, b) for b in range(8)]
    a2 = [("A2", s, b) for b in range(8)]
    if ORDER == "c":
        seq += a1[0:2]; take()
        seq += a1[2:4]; take()
        seq += a1[4:6] + a2[0:2]; take()
        seq += a1[6:8] + a2[2:4]; take()
        seq += a2[4:6]; take()
        seq += a2[6:8]
        while proj:
            take()
    elif ORDER == "f":
        for i in range(8):
            seq.append(a1[i])
            if i >= 2:
                seq.append(a2[i - 2])
            take()
        seq += a2[6:8]
        while proj:
            take()
    elif ORDER == "h":
        seq += a1[0:2]; take()
        seq += a1[2:4] + a2[0:2]; take()
        seq += a1[4:6] + a2[2:4]; take()
        seq += a1[6:8] + a2[4:6]; take()
        seq += a2[6:8]
        while proj:
            take()
    return seq


def build():
    if KHEAD:
        chunks = [("QK", 0, k) for k in range(4)]
    else:
        chunks = [("Q", 0, j) for j in range(NT)]
    for s in range(HKV + 1):
        chunks += stage(s)
    n = len(chunks)
    units = []
    for c in chunks:
        for u in needs(c):
            if u not in units:
                units.append(u)
    done = {}
    cum = 0.0
    for u in units:
        cum += UNIT_MB[u[0]]
        done[u] = DMA_L + cum / DMA_R
    first_need = {}
    for i, c in enumerate(chunks):
        for u in needs(c):
            first_need.setdefault(u, i)
    pref = [0.0]
    for c in chunks:
        pref.append(pref[-1] + CHUNK_US[c[0]])

    def arr(p, q):
        t = 0.0
        for u in units:
            if p <= first_need[u] < q:
                t = max(t, done[u])
        return t

    def cost(p):
        if p == 0:
            return 0.07
        if chunks[p - 1][0] in PROJ:
            c = C_PP if (p < 2 or chunks[p - 2][0] in PROJ) else C_AP
        else:
            c = C_A
        if chunks[p][0] == "A2":
            c += C_NEXT_A2
        return c

    INF = 1e18
    A = [INF] * (n + 1)
    prev = [None] * (n + 1)
    A[0] = 0.0
    for q in range(1, n + 1):
        for p in range(q):
            if A[p] >= INF:
                continue
            t = max(A[p], arr(p, q)) + cost(p) + pref[q] - pref[p]
            if t < A[q] - 1e-12:
                A[q] = t
                prev[q] = p
    pos = []
    q = n
    while q is not None and q > 0:
        p = prev[q]
        pos.append(p)
        q = p
    pos = sorted(pos)
    bounds = pos + [n]
    groups = []
    prog = []
    for bi, p in enumerate(pos):
        q = bounds[bi + 1]
        grp = [u for u in units if p <= first_need[u] < q]
        if grp:
            groups.append(grp)
            prog.append(("wait", len(groups) - 1))
        prog.extend(chunks[p:q])
    return units, groups, prog, A[n], [(p, chunks[p]) for p in pos]


UNITS, GROUPS, PROGRAM, EST_T, POS = build()
GROUP_OF = {u: gi for gi, g in enumerate(GROUPS) for u in g}
NSEM = len(GROUPS) + 1


def _kernel(x_hbm, k_hbm, v_hbm, wq_hbm, wo_hbm, out_hbm,
            x_v, k_v, v_v, wq_v, wo_v, q_scr, o_scr, acc_ref, ostage, sems):
    scale = DH ** -0.5

    def copy(u):
        s = sems.at[GROUP_OF[u]]
        if u[0] == "x":
            return pltpu.make_async_copy(x_hbm, x_v, s)
        if u[0] == "xk":
            return pltpu.make_async_copy(x_hbm.at[:, pl.ds(u[1] * DH, DH)], x_v.at[:, pl.ds(u[1] * DH, DH)], s)
        if u[0] == "wqk":
            return pltpu.make_async_copy(wq_hbm.at[pl.ds(u[1] * DH, DH), pl.ds(0, GW)],
                                         wq_v.at[0, pl.ds(u[1] * DH, DH), :], s)
        if u[0] == "wqt":
            _, g, j = u
            return pltpu.make_async_copy(wq_hbm.at[:, pl.ds(g * GW + j * DH, DH)], wq_v.at[g, :, pl.ds(j * DH, DH)], s)
        if u[0] == "wq":
            g = u[1]
            return pltpu.make_async_copy(wq_hbm.at[:, pl.ds(g * GW, GW)], wq_v.at[g], s)
        if u[0] == "wo":
            g = u[1]
            return pltpu.make_async_copy(wo_hbm.at[pl.ds(g * GW, GW), :], wo_v.at[g], s)
        if u[0] == "k":
            return pltpu.make_async_copy(k_hbm.at[:, u[1]], k_v.at[u[1]], s)
        if u[0] == "v":
            return pltpu.make_async_copy(v_hbm.at[:, u[1]], v_v.at[u[1]], s)
        raise ValueError(u)

    def out_copy(j):
        return pltpu.make_async_copy(ostage.at[j], out_hbm.at[:, pl.ds(j * DH, DH)], sems.at[NSEM - 1])

    def qk(k):
        part = jnp.dot(x_v[:, k * DH:(k + 1) * DH], wq_v[0, k * DH:(k + 1) * DH, :],
                       preferred_element_type=jnp.float32)
        if k == 0:
            acc_ref[...] = part
        elif k == 3:
            q_scr[:, 0:GW] = (acc_ref[...] + part).astype(jnp.bfloat16)
        else:
            acc_ref[...] += part

    def qc(g, j):
        c0 = (g * REP + j) * DH
        q_scr[:, c0:c0 + DH] = jnp.dot(
            x_v[...], wq_v[g, :, j * DH:(j + 1) * DH], preferred_element_type=jnp.float32
        ).astype(jnp.bfloat16)

    def oc(g, j):
        part = jnp.dot(o_scr[:, g * GW:(g + 1) * GW], wo_v[g, :, j * DH:(j + 1) * DH],
                       preferred_element_type=jnp.float32)
        if g == 0:
            acc_ref[:, j * DH:(j + 1) * DH] = part
        elif g == HKV - 1:
            ostage[j] = (acc_ref[:, j * DH:(j + 1) * DH] + part).astype(ostage.dtype)
            out_copy(j).start()
        else:
            acc_ref[:, j * DH:(j + 1) * DH] += part

    def a1(g, b):
        qs = jnp.concatenate(
            [q_scr[b * SQ:(b + 1) * SQ, (g * REP + j) * DH:(g * REP + j + 1) * DH] for j in range(REP)], axis=0)
        kb = k_v[g, b]
        st = lax.dot_general(kb, qs, (((1,), (1,)), ((), ())), preferred_element_type=jnp.float32)
        m = jnp.max(st, axis=0, keepdims=True)
        e = jnp.exp((st - m) * scale)
        l = jnp.sum(e, axis=0, keepdims=True)
        return (e * _recip(l)).astype(jnp.bfloat16)

    def a2(g, b, pt):
        vb = v_v[g, b]
        o = lax.dot_general(pt, vb, (((0,), (0,)), ((), ())), preferred_element_type=jnp.float32).astype(jnp.bfloat16)
        for j in range(REP):
            c0 = (g * REP + j) * DH
            o_scr[b * SQ:(b + 1) * SQ, c0:c0 + DH] = o[j * SQ:(j + 1) * SQ, :]

    for u in UNITS:
        copy(u).start()

    pts = {}
    for op in PROGRAM:
        if op[0] == "wait":
            for u in GROUPS[op[1]]:
                copy(u).wait()
        elif op[0] == "QK":
            qk(op[2])
        elif op[0] == "Q":
            qc(op[1], op[2])
        elif op[0] == "O":
            oc(op[1], op[2])
        elif op[0] == "A1":
            pts[(op[1], op[2])] = a1(op[1], op[2])
        elif op[0] == "A2":
            a2(op[1], op[2], pts.pop((op[1], op[2])))
    for j in range(NT):
        out_copy(j).wait()


@jax.jit
def pallas_standalone__gqa_block_cached__near_ridge_kernel(x, k_cache, v_cache, wq, wo):
    x2 = x.reshape(M, D)
    any_spec = pl.BlockSpec(memory_space=pl.ANY)
    out = pl.pallas_call(
        _kernel,
        grid_spec=pl.GridSpec(
            grid=(),
            in_specs=[any_spec] * 5,
            out_specs=any_spec,
            scratch_shapes=[
                pltpu.VMEM((M, D), jnp.bfloat16),
                pltpu.VMEM((HKV, B, SK, DH), jnp.bfloat16),
                pltpu.VMEM((HKV, B, SK, DH), jnp.bfloat16),
                pltpu.VMEM((HKV, D, GW), jnp.bfloat16),
                pltpu.VMEM((HKV, GW, D), jnp.bfloat16),
                pltpu.VMEM((M, HQ * DH), jnp.bfloat16),
                pltpu.VMEM((M, HQ * DH), jnp.bfloat16),
                pltpu.VMEM((M, D), jnp.float32),
                pltpu.VMEM((NT, M, DH), jnp.bfloat16),
                pltpu.SemaphoreType.DMA((NSEM,)),
            ],
        ),
        out_shape=jax.ShapeDtypeStruct((M, D), x.dtype),
        compiler_params=pltpu.CompilerParams(vmem_limit_bytes=100 * 1024 * 1024),
    )(x2, k_cache, v_cache, wq, wo)
    return out.reshape(B, SQ, D)
```

```python
import functools
import jax
import jax.numpy as jnp
from jax import lax
from jax.experimental import pallas as pl
from jax.experimental.pallas import tpu as pltpu

B, SQ, D = 8, 64, 512
HQ, HKV, SK, DH = 32, 8, 64, 128
REP = HQ // HKV
GW = REP * DH
M = B * SQ
NT = 4
NSPLIT = 4

DMA_L = 0.60
DMA_R = 0.66
ORDER = "c"
KHEAD = True
C_PP = 0.145
C_AP = 0.27
C_A = 0.37
C_NEXT_A2 = 0.15


def _recip(l):
    r = pl.reciprocal(l, approx=True)
    return r * (2.0 - l * r)


UNIT_MB = {"x": 0.5, "wqt": 0.125, "wq": 0.5, "wo": 0.5, "k": 0.125, "v": 0.125, "xk": 0.125, "wqk": 0.125}
CHUNK_US = {"Q": 512 / 1500.0, "O": 512 / 1500.0, "QK": 512 / 1500.0, "A1": 40 / 1500.0, "A2": 64 / 1500.0}
PROJ = ("Q", "O", "QK")


def needs(op):
    kind, g, j = op
    if kind == "QK":
        return [("xk", j), ("wqk", j)]
    if kind == "Q":
        if g == 0:
            return [("x",), ("wqt", 0, j)]
        return [("wq", g)]
    if kind == "O":
        return [("wo", g)]
    if kind == "A1":
        return [("k", g)]
    if kind == "A2":
        return [("v", g)]
    raise ValueError(op)


def stage(s):
    proj = []
    for j in range(NT):
        if s + 1 < HKV:
            proj.append(("Q", s + 1, j))
        if s >= 1:
            proj.append(("O", s - 1, j))
    if s == HKV:
        return proj
    seq = []
    take = lambda: seq.append(proj.pop(0)) if proj else None
    a1 = [("A1", s, b) for b in range(8)]
    a2 = [("A2", s, b) for b in range(8)]
    if ORDER == "c":
        seq += a1[0:2]; take()
        seq += a1[2:4]; take()
        seq += a1[4:6] + a2[0:2]; take()
        seq += a1[6:8] + a2[2:4]; take()
        seq += a2[4:6]; take()
        seq += a2[6:8]
        while proj:
            take()
    elif ORDER == "f":
        for i in range(8):
            seq.append(a1[i])
            if i >= 2:
                seq.append(a2[i - 2])
            take()
        seq += a2[6:8]
        while proj:
            take()
    elif ORDER == "h":
        seq += a1[0:2]; take()
        seq += a1[2:4] + a2[0:2]; take()
        seq += a1[4:6] + a2[2:4]; take()
        seq += a1[6:8] + a2[4:6]; take()
        seq += a2[6:8]
        while proj:
            take()
    return seq


def build():
    if KHEAD:
        chunks = [("QK", 0, k) for k in range(4)]
    else:
        chunks = [("Q", 0, j) for j in range(NT)]
    for s in range(HKV + 1):
        chunks += stage(s)
    n = len(chunks)
    units = []
    for c in chunks:
        for u in needs(c):
            if u not in units:
                units.append(u)
    done = {}
    cum = 0.0
    for u in units:
        cum += UNIT_MB[u[0]]
        done[u] = DMA_L + cum / DMA_R
    first_need = {}
    for i, c in enumerate(chunks):
        for u in needs(c):
            first_need.setdefault(u, i)
    pref = [0.0]
    for c in chunks:
        pref.append(pref[-1] + CHUNK_US[c[0]])

    def arr(p, q):
        t = 0.0
        for u in units:
            if p <= first_need[u] < q:
                t = max(t, done[u])
        return t

    def cost(p):
        if p == 0:
            return 0.07
        if chunks[p - 1][0] in PROJ:
            c = C_PP if (p < 2 or chunks[p - 2][0] in PROJ) else C_AP
        else:
            c = C_A
        if chunks[p][0] == "A2":
            c += C_NEXT_A2
        return c

    INF = 1e18
    A = [INF] * (n + 1)
    prev = [None] * (n + 1)
    A[0] = 0.0
    for q in range(1, n + 1):
        for p in range(q):
            if A[p] >= INF:
                continue
            t = max(A[p], arr(p, q)) + cost(p) + pref[q] - pref[p]
            if t < A[q] - 1e-12:
                A[q] = t
                prev[q] = p
    pos = []
    q = n
    while q is not None and q > 0:
        p = prev[q]
        pos.append(p)
        q = p
    pos = sorted(pos)
    bounds = pos + [n]
    groups = []
    prog = []
    for bi, p in enumerate(pos):
        q = bounds[bi + 1]
        grp = [u for u in units if p <= first_need[u] < q]
        if grp:
            groups.append(grp)
            prog.append(("wait", len(groups) - 1))
        prog.extend(chunks[p:q])
    return units, groups, prog, A[n], [(p, chunks[p]) for p in pos]


UNITS, GROUPS, PROGRAM, EST_T, POS = build()
GROUP_OF = {u: gi for gi, g in enumerate(GROUPS) for u in g}
NSEM = len(GROUPS) + 1


def _kernel(x_hbm, k_hbm, v_hbm, wq_hbm, wo_hbm, out_hbm,
            x_v, k_v, v_v, wq_v, wo_v, q_scr, o_scr, acc_ref, ostage, sems):
    scale = DH ** -0.5

    def copy(u):
        s = sems.at[GROUP_OF[u]]
        if u[0] == "x":
            return pltpu.make_async_copy(x_hbm, x_v, s)
        if u[0] == "xk":
            return pltpu.make_async_copy(x_hbm.at[:, pl.ds(u[1] * DH, DH)], x_v.at[:, pl.ds(u[1] * DH, DH)], s)
        if u[0] == "wqk":
            return pltpu.make_async_copy(wq_hbm.at[pl.ds(u[1] * DH, DH), pl.ds(0, GW)],
                                         wq_v.at[0, pl.ds(u[1] * DH, DH), :], s)
        if u[0] == "wqt":
            _, g, j = u
            return pltpu.make_async_copy(wq_hbm.at[:, pl.ds(g * GW + j * DH, DH)], wq_v.at[g, :, pl.ds(j * DH, DH)], s)
        if u[0] == "wq":
            g = u[1]
            return pltpu.make_async_copy(wq_hbm.at[:, pl.ds(g * GW, GW)], wq_v.at[g], s)
        if u[0] == "wo":
            g = u[1]
            return pltpu.make_async_copy(wo_hbm.at[pl.ds(g * GW, GW), :], wo_v.at[g], s)
        if u[0] == "k":
            return pltpu.make_async_copy(k_hbm.at[:, u[1]], k_v.at[u[1]], s)
        if u[0] == "v":
            return pltpu.make_async_copy(v_hbm.at[:, u[1]], v_v.at[u[1]], s)
        raise ValueError(u)

    def out_copy(j, r=None):
        if r is None:
            return pltpu.make_async_copy(ostage.at[j], out_hbm.at[:, pl.ds(j * DH, DH)], sems.at[NSEM - 1])
        rows = pl.ds(r * (M // NSPLIT), M // NSPLIT)
        return pltpu.make_async_copy(ostage.at[j, rows], out_hbm.at[rows, pl.ds(j * DH, DH)], sems.at[NSEM - 1])

    def qk(k):
        part = jnp.dot(x_v[:, k * DH:(k + 1) * DH], wq_v[0, k * DH:(k + 1) * DH, :],
                       preferred_element_type=jnp.float32)
        if k == 0:
            acc_ref[...] = part
        elif k == 3:
            q_scr[:, 0:GW] = (acc_ref[...] + part).astype(jnp.bfloat16)
        else:
            acc_ref[...] += part

    def qc(g, j):
        c0 = (g * REP + j) * DH
        q_scr[:, c0:c0 + DH] = jnp.dot(
            x_v[...], wq_v[g, :, j * DH:(j + 1) * DH], preferred_element_type=jnp.float32
        ).astype(jnp.bfloat16)

    def oc(g, j):
        if g == HKV - 1 and j == NT - 1:
            rb = M // NSPLIT
            for r in range(NSPLIT):
                part = jnp.dot(o_scr[r * rb:(r + 1) * rb, g * GW:(g + 1) * GW], wo_v[g, :, j * DH:(j + 1) * DH],
                               preferred_element_type=jnp.float32)
                ostage[j, r * rb:(r + 1) * rb, :] = (
                    acc_ref[r * rb:(r + 1) * rb, j * DH:(j + 1) * DH] + part).astype(ostage.dtype)
                out_copy(j, r).start()
            return
        part = jnp.dot(o_scr[:, g * GW:(g + 1) * GW], wo_v[g, :, j * DH:(j + 1) * DH],
                       preferred_element_type=jnp.float32)
        if g == 0:
            acc_ref[:, j * DH:(j + 1) * DH] = part
        elif g == HKV - 1:
            ostage[j] = (acc_ref[:, j * DH:(j + 1) * DH] + part).astype(ostage.dtype)
            out_copy(j).start()
        else:
            acc_ref[:, j * DH:(j + 1) * DH] += part

    def a1(g, b):
        qs = jnp.concatenate(
            [q_scr[b * SQ:(b + 1) * SQ, (g * REP + j) * DH:(g * REP + j + 1) * DH] for j in range(REP)], axis=0)
        kb = k_v[g, b]
        st = lax.dot_general(kb, qs, (((1,), (1,)), ((), ())), preferred_element_type=jnp.float32)
        m = jnp.max(st, axis=0, keepdims=True)
        e = jnp.exp((st - m) * scale)
        l = jnp.sum(e, axis=0, keepdims=True)
        return (e * _recip(l)).astype(jnp.bfloat16)

    def a2(g, b, pt):
        vb = v_v[g, b]
        o = lax.dot_general(pt, vb, (((0,), (0,)), ((), ())), preferred_element_type=jnp.float32).astype(jnp.bfloat16)
        for j in range(REP):
            c0 = (g * REP + j) * DH
            o_scr[b * SQ:(b + 1) * SQ, c0:c0 + DH] = o[j * SQ:(j + 1) * SQ, :]

    for u in UNITS:
        copy(u).start()

    pts = {}
    for op in PROGRAM:
        if op[0] == "wait":
            for u in GROUPS[op[1]]:
                copy(u).wait()
        elif op[0] == "QK":
            qk(op[2])
        elif op[0] == "Q":
            qc(op[1], op[2])
        elif op[0] == "O":
            oc(op[1], op[2])
        elif op[0] == "A1":
            pts[(op[1], op[2])] = a1(op[1], op[2])
        elif op[0] == "A2":
            a2(op[1], op[2], pts.pop((op[1], op[2])))
    for j in range(NT - 1):
        out_copy(j).wait()
    for r in range(NSPLIT):
        out_copy(NT - 1, r).wait()


@jax.jit
def pallas_standalone__gqa_block_cached__near_ridge_kernel(x, k_cache, v_cache, wq, wo):
    x2 = x.reshape(M, D)
    any_spec = pl.BlockSpec(memory_space=pl.ANY)
    out = pl.pallas_call(
        _kernel,
        grid_spec=pl.GridSpec(
            grid=(),
            in_specs=[any_spec] * 5,
            out_specs=any_spec,
            scratch_shapes=[
                pltpu.VMEM((M, D), jnp.bfloat16),
                pltpu.VMEM((HKV, B, SK, DH), jnp.bfloat16),
                pltpu.VMEM((HKV, B, SK, DH), jnp.bfloat16),
                pltpu.VMEM((HKV, D, GW), jnp.bfloat16),
                pltpu.VMEM((HKV, GW, D), jnp.bfloat16),
                pltpu.VMEM((M, HQ * DH), jnp.bfloat16),
                pltpu.VMEM((M, HQ * DH), jnp.bfloat16),
                pltpu.VMEM((M, D), jnp.float32),
                pltpu.VMEM((NT, M, DH), jnp.bfloat16),
                pltpu.SemaphoreType.DMA((NSEM,)),
            ],
        ),
        out_shape=jax.ShapeDtypeStruct((M, D), x.dtype),
        compiler_params=pltpu.CompilerParams(vmem_limit_bytes=100 * 1024 * 1024),
    )(x2, k_cache, v_cache, wq, wo)
    return out.reshape(B, SQ, D)
```
